```python
import os as _os
_os.environ.setdefault("JAX_PLATFORMS", "cpu")
import jax
import jax.numpy as jnp

def _softmax(x, axis=-1):
    return jax.nn.softmax(x, axis=axis)
def _gelu(x):
    return jax.nn.gelu(x, approximate=True)
def _silu(x):
    return jax.nn.silu(x)
def _sigmoid(x):
    return jax.nn.sigmoid(x)
def _layernorm(x, axis=-1, eps=1e-5):
    m = jnp.mean(x, axis=axis, keepdims=True)
    v = jnp.var(x, axis=axis, keepdims=True)
    return (x - m) / jnp.sqrt(v + eps)
def _scatter_add(tgt, idx, src, axis=0):
    return tgt.at[idx].add(src)
def _segment_sum(src, seg, n):
    return jax.ops.segment_sum(src, seg, n)
class _Rng:
    def __init__(self, key):
        self._k = key
    def _next(self):
        self._k, sub = jax.random.split(self._k)
        return sub
    def normal(self, shape):
        return jax.random.normal(self._next(), shape, dtype=jnp.bfloat16)
    def randint(self, lo, hi, shape):
        return jax.random.randint(self._next(), shape, lo, hi, dtype=jnp.int32)
    def uniform(self, shape, lo=0.0, hi=1.0):
        return jax.random.uniform(self._next(), shape, jnp.bfloat16, lo, hi)
    def permutation(self, n):
        return jax.random.permutation(self._next(), n)


kernel_name = 'parallel_sum__sliding_local_dilated__dense_activation_mish__prompt'

def setup_inputs():
    _rng = _Rng(jax.random.key(int.from_bytes(__import__("os").urandom(4), "little")))
    _w = (lambda a: (lambda t: t.astype(jnp.bfloat16) if jnp.issubdtype(t.dtype, jnp.floating) else t)(jnp.asarray(a)))
    def _A_setup():
        B, S, D = 1, 2048, 576
        return {
            "x": _w((lambda *s: _rng.normal(s) * 0.05)(B, S, D)),
            "wqkv": _w((lambda *s: _rng.normal(s) * 0.05)(D, 3 * D)),
            "wo": _w((lambda *s: _rng.normal(s) * 0.05)(D, D)),
        }
    _A_in = _A_setup()

    def _B_setup():
        B, S, D, F = 1, 2048, 576, 4608
        return {
            "x": _w((lambda *s: _rng.normal(s) * 0.05)(B, S, D)),
            "w1": _w((lambda *s: _rng.normal(s) * 1.6)(D, F) * (D ** -0.5)),
            "b1": _w((lambda *s: _rng.normal(s) * 0.2)(F)),
            "w2": _w((lambda *s: _rng.normal(s) * 0.2)(F, D) * (F ** -0.5)),
        }
    _B_in = _B_setup()

    return {
        "A_x": _A_in["x"],
        "A_wqkv": _A_in["wqkv"],
        "A_wo": _A_in["wo"],
        "B_x": _B_in["x"],
        "B_w1": _B_in["w1"],
        "B_b1": _B_in["b1"],
        "B_w2": _B_in["w2"],
    }

def reference(A_x, A_wqkv, A_wo, B_x, B_w1, B_b1, B_w2):
    def _A_ref(x, wqkv, wo):
        B, S, D = x.shape
        H = 32; Dh = D // H
        W, dil = 8, 2
        qkv = (lambda x, *d: x.transpose(*d))((x @ wqkv).reshape(B, S, 3, H, Dh), 2, 0, 3, 1, 4)
        q, k, v = qkv[0], qkv[1], qkv[2]
        scale = Dh ** -0.5
        pos = jnp.arange(S)
        off = jnp.arange(W) * dil
        idx = pos[:, None] - off[None, :]
        mask = idx >= 0
        idx_c = jnp.where(mask, idx, 0).reshape(-1)
        kg = k[:, :, idx_c, :].reshape(B, H, S, W, Dh)
        vg = v[:, :, idx_c, :].reshape(B, H, S, W, Dh)
        logits = jnp.einsum("bhsd,bhswd->bhsw", q, kg) * scale
        logits = jnp.where(mask[None, None, :, :], logits, -1e9)
        attn = _softmax(logits, axis=-1)
        o = jnp.einsum("bhsw,bhswd->bhsd", attn, vg)
        return (lambda x, *d: x.transpose(*d))(o, 0, 2, 1, 3).reshape(B, S, D) @ wo

    def _B_ref(x, w1, b1, w2):
        h = jnp.einsum("bsd,df->bsf", x, w1) + b1
        sp = jnp.log1p(jnp.exp(-jnp.abs(h))) + jnp.where(h > 0, h, jnp.zeros_like(h))
        act = h * jnp.tanh(sp)
        return jnp.einsum("bsf,fd->bsd", act, w2)

    x = A_x
    xn = _layernorm(x, axis=-1)
    return x + _A_ref(xn, A_wqkv, A_wo) + _B_ref(xn, B_w1, B_b1, B_w2)
```

```python
import functools, math
import jax
import jax.numpy as jnp
import jax.experimental.pallas as pl
import jax.experimental.pallas.tpu as pltpu

S, D, F = 2048, 576, 4608
H, DH, W, DIL = 32, 18, 8, 2
KP = 640
NQKV = 14 * 128
HALO = 16
LOG2E = 1.4426950408889634
LN2 = 0.6931471805599453
EPS = 1e-5
L2E_HI = 1.4453125
L2E_LO = -0.00262451171875
NT = (((1,), (1,)), ((), ()))
RB = 256
NB = S // RB
NM = 8
TFM = 512
SCOPES = False


class _Null:
    def __enter__(self): return self
    def __exit__(self, *a): return False


def scope(name):
    return jax.named_scope(name) if SCOPES else _Null()


def make_kernel(TF0, RC, sched):
    TFL = F - TF0 - NM * TFM
    nrc = RB // RC
    SX, SW1, SW2, SWQ, SWO, SB, SO = 0, NB, NB + NM + 2, NB + 2 * NM + 4, NB + 2 * NM + 5, NB + 2 * NM + 6, NB + 2 * NM + 7

    def kernel(xt_hbm, wqkv_hbm, wo_hbm, w1_hbm, b1_hbm, w2t_hbm, out_hbm,
               xbuf, xn_ref, w1f, w1m, w1l, w2f, w2m, w2l, wq_raw, wo_raw, b1_ref, wp_ref, wotp_ref,
               t_ref, wo32_ref, acc_ref, acca_ref, obuf, kv_ref, q_ref, oa_ref, fz_ref, zs_ref, sems):
        step = pl.program_id(0)

        def x_copy(i):
            return pltpu.make_async_copy(xt_hbm.at[:, pl.ds(i * RB, RB)], xbuf.at[i], sems.at[SX + i])

        def o_copy(i):
            return pltpu.make_async_copy(obuf.at[i], out_hbm.at[:, pl.ds(i * RB, RB)], sems.at[SO + i])

        def w_first():
            return (pltpu.make_async_copy(w1_hbm.at[:, pl.ds(0, TF0)], w1f.at[pl.ds(0, D), :], sems.at[SW1]),
                    pltpu.make_async_copy(w2t_hbm.at[:, pl.ds(0, TF0)], w2f, sems.at[SW2]))

        def w_mid(c):
            off = TF0 + c * TFM
            if not isinstance(c, int):
                off = pl.multiple_of(off, 128)
            return (pltpu.make_async_copy(w1_hbm.at[:, pl.ds(off, TFM)], w1m.at[c, pl.ds(0, D), :], sems.at[SW1 + 1 + c]),
                    pltpu.make_async_copy(w2t_hbm.at[:, pl.ds(off, TFM)], w2m.at[c], sems.at[SW2 + 1 + c]))

        def w_last():
            return (pltpu.make_async_copy(w1_hbm.at[:, pl.ds(F - TFL, TFL)], w1l.at[pl.ds(0, D), :], sems.at[SW1 + NM + 1]),
                    pltpu.make_async_copy(w2t_hbm.at[:, pl.ds(F - TFL, TFL)], w2l, sems.at[SW2 + NM + 1]))

        wq_copy = pltpu.make_async_copy(wqkv_hbm, wq_raw, sems.at[SWQ])
        wo_copy = pltpu.make_async_copy(wo_hbm, wo_raw, sems.at[SWO])
        b1_copy = pltpu.make_async_copy(b1_hbm, b1_ref, sems.at[SB])

        def prep_wqkv1():
            wq = pltpu.bitcast(wq_raw[...], jnp.uint32)
            wq = jnp.concatenate([wq, jnp.zeros((384 - 288, 3 * D), jnp.uint32)], axis=0)
            wq = jnp.concatenate([wq, jnp.zeros((384, NQKV - 3 * D), jnp.uint32)], axis=1)
            for j in range(3):
                t_ref[j] = wq[j * 128:(j + 1) * 128, :].T

        def prep_wqkv2():
            for j in range(3):
                g = lambda x, d: t_ref[j, pl.ds(x * D + d, H, stride=DH), :]
                parts = [g(x, d) for x in range(3) for d in range(16)]
                parts += [g(0, 16), g(0, 17), jnp.zeros((64, 128), jnp.uint32), g(1, 16), g(1, 17), g(2, 16), g(2, 17)]
                blk = jnp.concatenate(parts, axis=0).T
                n = 128 if j < 2 else 32
                wp_ref[j * 256:j * 256 + 2 * n, :] = pltpu.bitcast(blk[:n], jnp.bfloat16)
            wp_ref[D:KP, :] = jnp.zeros((KP - D, NQKV), jnp.bfloat16)

        def prep_wo():
            wo = wo_raw[...].astype(jnp.float32)
            wo = jnp.concatenate([wo, jnp.zeros((D, KP - D), jnp.float32)], axis=1)
            for j in range(5):
                wo32_ref[j] = wo[:, j * 128:(j + 1) * 128]
            for j in range(5):
                g = lambda d: wo32_ref[j, pl.ds(d, H, stride=DH), :]
                parts = [g(d) for d in range(16)] + [jnp.zeros((64, 128), jnp.float32), g(16), g(17)]
                n = 128 if j < 4 else 64
                blk = jnp.concatenate(parts, axis=0).T
                wotp_ref[j * 128:j * 128 + n, :] = blk[:n].astype(jnp.bfloat16)

        def bias_rows(off, n):
            r = jax.lax.broadcasted_iota(jnp.int32, (KP - D, n), 0)
            b = b1_ref[pl.ds(off, n)].astype(jnp.float32).reshape(1, n)
            return jnp.where(r < 2, jnp.broadcast_to(b, (KP - D, n)), 0.0).astype(jnp.bfloat16)

        def prep_bias_rest():
            for c in range(NM):
                w1m[c, D:KP, :] = bias_rows(TF0 + c * TFM, TFM)
            w1l[D:KP, :] = bias_rows(F - TFL, TFL)

        def ln_prep(b):
            x = xbuf[b].astype(jnp.float32)
            mu = jnp.sum(x, axis=0, keepdims=True) * (1.0 / D)
            xc = x - mu
            var = jnp.sum(xc * xc, axis=0, keepdims=True) * (1.0 / D)
            xn = xc * (jax.lax.rsqrt(var + EPS) * LOG2E)
            r = jax.lax.broadcasted_iota(jnp.int32, (KP - D, RB), 0)
            pad = jnp.where(r == 0, L2E_HI, jnp.where(r == 1, L2E_LO, 0.0))
            xn = jnp.concatenate([xn, pad], axis=0)
            xn_ref[b] = xn.T.astype(jnp.bfloat16)

        def attn(r0, j):
            qs = fz_ref[1]
            qs = jnp.concatenate([qs] * (RC // 8), axis=0)
            q = [q_ref[i, r0:r0 + RC, :] * qs for i in range(5)]
            logits = []
            for w in range(W):
                lo = HALO + r0 - DIL * w
                p = q[0] * kv_ref[0, lo:lo + RC, :]
                for i in range(1, 4):
                    p = p + q[i] * kv_ref[i, lo:lo + RC, :]
                p = p + q[4] * kv_ref[8, lo:lo + RC, :]
                p = p + pltpu.roll(p, 64, 1)
                p = p + pltpu.roll(p, 32, 1)
                if r0 < DIL * w:
                    pos = j * RB + r0 + jax.lax.broadcasted_iota(jnp.int32, (RC, 128), 0)
                    p = jnp.where(pos >= DIL * w, p, -1e9)
                logits.append(p)
            m = logits[0]
            for w in range(1, W):
                m = jnp.maximum(m, logits[w])
            e = [jnp.exp2(l - m) for l in logits]
            den = e[0]
            for w in range(1, W):
                den = den + e[w]
            inv = 1.0 / den
            for i in range(5):
                pi = 4 + i if i < 4 else 8
                acc = None
                for w in range(W):
                    lo = HALO + r0 - DIL * w
                    t = e[w] * kv_ref[pi, lo:lo + RC, :]
                    acc = t if acc is None else acc + t
                oa_ref[r0:r0 + RC, i * 128:(i + 1) * 128] = (acc * inv).astype(jnp.bfloat16)

        def mish(h):
            e = jnp.exp2(jnp.minimum(h, 30.0))
            n = e * (e + 2.0)
            return ((h * n) * pl.reciprocal(n + 2.0, approx=True)).astype(jnp.bfloat16)

        def m1(b, w1c):
            return mish(jnp.dot(xn_ref[b], w1c, preferred_element_type=jnp.float32))

        def m2(act, w2c):
            return jax.lax.dot_general(w2c, act, NT, preferred_element_type=jnp.float32)

        def first():
            w1c, w2c = w_first()
            wm1, wm2 = w_mid(0)
            cps = {'w1': w1c, 'w2': w2c, 'wq': wq_copy, 'wo': wo_copy, 'b1': b1_copy, 'm1': wm1, 'm2': wm2}
            for i in range(NB):
                cps['x%d' % i] = x_copy(i)
            order, prog = sched
            for name in order.split():
                cps[name].start()
            zs_ref[0] = 0
            fz_ref[1] = jnp.full((8, 128), (DH ** -0.5) / LOG2E, jnp.float32)
            kv_ref[:, RB:RB + HALO, :] = jnp.zeros((9, HALO, 128), jnp.float32)
            acts = {}
            for tok in prog.split():
                if tok[0] == '!':
                    with scope("wait_" + tok[1:]):
                        for name in tok[1:].split(','):
                            cps[name].wait()
                elif tok[0] == 'L':
                    ln_prep(int(tok[1:]))
                elif tok[0] == 'A':
                    acts[int(tok[1:])] = m1(int(tok[1:]), w1f[...])
                elif tok[0] == 'H':
                    acts[int(tok[1:])] = jnp.dot(xn_ref[int(tok[1:])], w1f[...], preferred_element_type=jnp.float32)
                elif tok[0] == 'M':
                    acts[int(tok[1:])] = mish(acts[int(tok[1:])])
                elif tok[0] == 'B':
                    acc_ref[int(tok[1:])] = m2(acts.pop(int(tok[1:])), w2f[...])
                elif tok == 'bias0':
                    w1f[D:KP, :] = bias_rows(0, TF0)
                elif tok == 'biasr':
                    prep_bias_rest()
                elif tok == 'P1':
                    prep_wqkv1()
                elif tok == 'P2':
                    prep_wqkv2()
                elif tok == 'PO':
                    prep_wo()
                else:
                    raise ValueError(tok)

        def mid():
            c = step - 1
            for cp in w_mid(c):
                cp.wait()

            @pl.when(c < NM - 1)
            def _():
                for cp in w_mid(c + 1):
                    cp.start()

            @pl.when(c == NM - 1)
            def _():
                for cp in w_last():
                    cp.start()

            z = zs_ref[0]
            kv_ref[:, 0:HALO, :] = kv_ref[:, RB:RB + HALO, :]
            qkv = jnp.dot(xn_ref[c], wp_ref[...], preferred_element_type=jnp.float32)
            for i in range(4):
                q_ref[i] = qkv[:, i * 128:(i + 1) * 128]
                kv_ref[i, HALO:HALO + RB, :] = qkv[:, 512 + i * 128:512 + (i + 1) * 128]
                kv_ref[4 + i, HALO:HALO + RB, :] = qkv[:, 1024 + i * 128:1024 + (i + 1) * 128]
            q_ref[4] = qkv[:, 1536:1664]
            kv_ref[8, HALO:HALO + RB, :] = qkv[:, 1664:1792]
            na = NB - 1

            def attn_group(g):
                for rc in range(g * nrc // na, (g + 1) * nrc // na):
                    attn(rc * RC, c)

            attn_group(0)
            act = m1(0, w1m[c])
            for b in range(NB):
                if b + 1 < NB:
                    nact = m1(b + 1, w1m[c])
                else:
                    acca_ref[c] = jax.lax.dot_general(wotp_ref[...], oa_ref[...], NT, preferred_element_type=jnp.float32)
                t = m2(act, w2m[c])
                acc_ref[b] = acc_ref[b] + t
                if b + 1 < na:
                    fz_ref[z] = t[0:8, 0:128]
                    attn_group(b + 1)
                act = nact

        def last():
            for cp in w_last():
                cp.wait()
            act = m1(0, w1l[...])
            for b in range(NB):
                if b + 1 < NB:
                    nact = m1(b + 1, w1l[...])
                if b >= 1:
                    o_copy(b - 1).start()
                t = m2(act, w2l[...])
                obuf[b] = (xbuf[b].astype(jnp.float32) + (acc_ref[b] + acca_ref[b] + t) * LN2).astype(jnp.bfloat16)
                act = nact
            o_copy(NB - 1).start()
            for b in range(NB):
                o_copy(b).wait()

        @pl.when(step == 0)
        def _():
            with scope("first"):
                first()

        @pl.when(jnp.logical_and(step > 0, step <= NM))
        def _():
            with scope("mid"):
                mid()

        @pl.when(step == NM + 1)
        def _():
            with scope("last"):
                last()

    return kernel, TFL


SCHEDS = {
    0: ("x0 b1 w1 w2 x1 x2 x3 x4 x5 wq x6 x7 wo m1 m2",
        "!x0 L0 !b1,w1 bias0 A0 !w2,x1 L1 biasr B0 !x2 L2 A1 A2 !x3,x4,x5 L3 L4 L5 B1 A3 B2 A4 !wq P1 B3 A5 B4 "
        "!x6,x7,wo L6 L7 P2 PO B5 A6 A7 B6 B7"),
    1: ("x0 b1 w1 x1 w2 x2 x3 wq x4 x5 x6 x7 wo m1 m2",
        "!x0 L0 !b1,w1,x1 bias0 L1 A0 H1 !w2,x2,x3 M1 L2 L3 biasr B0 A2 B1 A3 B2 !wq,x4,x5 L4 L5 P1 B3 A4 A5 B4 "
        "!x6,x7,wo L6 L7 P2 PO B5 A6 A7 B6 B7"),
    2: ("x0 b1 w1 x1 w2 x2 x3 wq x4 x5 x6 x7 wo m1 m2",
        "!x0 L0 !b1,w1 bias0 H0 !x1,w2 M0 L1 B0 H1 !x2,x3 M1 L2 L3 biasr B1 A2 A3 B2 !wq,x4,x5 L4 L5 P1 B3 A4 A5 B4 "
        "!x6,x7,wo L6 L7 P2 PO B5 A6 A7 B6 B7"),
}


_KERNEL, _TFL = make_kernel(384, 16, SCHEDS[2])
_TF0 = 384


@jax.jit
def pallas_parallel_sum__sliding_local_dilated__dense_activation_mish__prompt_kernel(
    A_x: jax.Array,
    A_wqkv: jax.Array,
    A_wo: jax.Array,
    B_x: jax.Array,
    B_w1: jax.Array,
    B_b1: jax.Array,
    B_w2: jax.Array,
):
    TF0, TFL = _TF0, _TFL
    kernel = _KERNEL
    xt = A_x.reshape(S, D).T
    w2t = B_w2.T
    hbm = pl.BlockSpec(memory_space=pl.ANY)
    bf, f32 = jnp.bfloat16, jnp.float32
    out_t = pl.pallas_call(
        kernel,
        grid=(NM + 2,),
        in_specs=[hbm] * 6,
        out_specs=hbm,
        out_shape=jax.ShapeDtypeStruct((D, S), bf),
        scratch_shapes=[
            pltpu.VMEM((NB, D, RB), bf),
            pltpu.VMEM((NB, RB, KP), bf),
            pltpu.VMEM((KP, TF0), bf), pltpu.VMEM((NM, KP, TFM), bf), pltpu.VMEM((KP, TFL), bf),
            pltpu.VMEM((D, TF0), bf), pltpu.VMEM((NM, D, TFM), bf), pltpu.VMEM((D, TFL), bf),
            pltpu.VMEM((D, 3 * D), bf),
            pltpu.VMEM((D, D), bf),
            pltpu.VMEM((F,), bf),
            pltpu.VMEM((KP, NQKV), bf),
            pltpu.VMEM((D, KP), bf),
            pltpu.VMEM((3, NQKV, 128), jnp.uint32),
            pltpu.VMEM((5, D, 128), f32),
            pltpu.VMEM((NB, D, RB), f32),
            pltpu.VMEM((NB, D, RB), f32),
            pltpu.VMEM((NB, D, RB), bf),
            pltpu.VMEM((9, RB + HALO, 128), f32),
            pltpu.VMEM((5, RB, 128), f32),
            pltpu.VMEM((RB, KP), bf),
            pltpu.VMEM((2, 8, 128), f32),
            pltpu.SMEM((1,), jnp.int32),
            pltpu.SemaphoreType.DMA((NB + 2 * NM + 7 + NB,)),
        ],
        compiler_params=pltpu.CompilerParams(
            dimension_semantics=("arbitrary",), vmem_limit_bytes=100 * 1024 * 1024),
        name="fused",
    )(xt, A_wqkv, A_wo, B_w1, B_b1, w2t)
    return out_t.T.reshape(1, S, D)
```

```python
import jax
import jax.numpy as jnp
import jax.experimental.pallas as pl
import jax.experimental.pallas.tpu as pltpu

S, D, F = 2048, 576, 4608
H, DH, W, DIL = 32, 18, 8, 2
KP = 640
NQ = 14 * 128
HALO = 16
RB = 256
NB = S // RB
TF = 512
NM = F // TF - 1
RC = 16
EPS = 1e-5
LOG2E = 1.4426950408889634
LN2 = 0.6931471805599453
L2E_HI = 1.4453125
L2E_LO = -0.00262451171875
NT = (((1,), (1,)), ((), ()))
F32, BF16, U32 = jnp.float32, jnp.bfloat16, jnp.uint32

RELEASE = [1, 1, 1, 1, 1, 0, 1, 1, 1] + [0, 1, 1, 0] * 4
REL_ROWS = (96, 400)

SX = 0
SW1 = SX + NB
SW2 = SW1 + NM + 2
SWQ = SW2 + NM + 2
SWO, SB, SO = SWQ + 1, SWQ + 2, SWQ + 3
NSEM = SO + NB + 1


def _pk(v):
    return pltpu.bitcast(v, U32)


def _upk(v):
    return pltpu.bitcast(v, BF16)


def _kernel(xt_hbm, wqkv_hbm, wo_hbm, w1_hbm, b1_hbm, w2t_hbm, out_hbm,
            xbuf, xn_ref, w1f, w1m, w2f, w2m, wq_raw, wo_raw, b1_ref, wp_ref, wotp_ref,
            t_ref, wo32_ref, acc_ref, obuf, kv_ref, q_ref, oa_ref, fz_ref, zs_ref, sems):
    step = pl.program_id(0)
    copy = pltpu.make_async_copy

    def x_copy(i):
        return copy(xt_hbm.at[:, pl.ds(i * RB, RB)], xbuf.at[i], sems.at[SX + i])

    def o_copy(i):
        return copy(obuf.at[i], out_hbm.at[:, pl.ds(i * RB, RB)], sems.at[SO + i])

    def o_half(i):
        hb = RB // 2
        return copy(obuf.at[NB - 1, :, pl.ds(i * hb, hb)],
                    out_hbm.at[:, pl.ds((NB - 1) * RB + i * hb, hb)], sems.at[SO + NB - 1 + i])

    def w1_first(i):
        cs = pl.ds(i * (TF // 2), TF // 2)
        return copy(w1_hbm.at[:, cs], w1f.at[pl.ds(0, D), cs], sems.at[SW1 + NM + i])

    def w2_first(i):
        cs = pl.ds(i * (TF // 2), TF // 2)
        return copy(w2t_hbm.at[:, cs], w2f.at[:, cs], sems.at[SW2 + NM + i])

    def w_mid(c):
        off = TF + c * TF
        if not isinstance(c, int):
            off = pl.multiple_of(off, 128)
        return (copy(w1_hbm.at[:, pl.ds(off, TF)], w1m.at[c, pl.ds(0, D), :], sems.at[SW1 + c]),
                copy(w2t_hbm.at[:, pl.ds(off, TF)], w2m.at[c], sems.at[SW2 + c]))

    def release(v):
        fz_ref[zs_ref[0]] = v

    def prep_wqkv(j):
        one = fz_ref[2, 0:1, 0:1]
        if j < 2:
            lo = wq_raw[j * 256:j * 256 + 128, :].astype(F32) * one
            hi = wq_raw[j * 256 + 128:j * 256 + 256, :].astype(F32)
            wq = _pk(pltpu.pack_elementwise([lo, hi], packed_dtype=BF16))
        else:
            hi = wq_raw[512:D, :].astype(F32) * one
            wq = jnp.concatenate([_pk(hi), jnp.zeros((64, 3 * D), U32)], axis=0)
        wq = jnp.concatenate([wq, jnp.zeros((128, NQ - 3 * D), U32)], axis=1)
        t_ref[j] = wq.T
        rows = lambda x, d: t_ref[j, pl.ds(x * D + d, H, stride=DH), :]
        parts = [rows(x, d) for x in range(3) for d in range(16)]
        parts += [rows(x, d) for x in range(3) for d in (16, 17)]
        u = jnp.concatenate(parts, axis=0)
        if j < 2:
            tiles = [(2 * j, pltpu.bitcast(u << 16, F32)),
                     (2 * j + 1, pltpu.bitcast(u & jnp.uint32(0xFFFF0000), F32))]
        else:
            tiles = [(4, pltpu.bitcast(u, F32))]
        for kt, v in tiles:
            wp_ref[:, kt * 128:(kt + 1) * 128] = _pk(v.astype(BF16))

    def prep_wo():
        wo = wo_raw[...].astype(F32) * fz_ref[2, 0:1, 0:1]
        wo = jnp.concatenate([wo, jnp.zeros((D, KP - D), F32)], axis=1)
        for j in range(5):
            wo32_ref[j] = wo[:, j * 128:(j + 1) * 128]
        for j in range(5):
            rows = lambda d: wo32_ref[j, pl.ds(d, H, stride=DH), :]
            parts = [rows(d) for d in range(16)] + [jnp.zeros((64, 128), F32), rows(16), rows(17)]
            n = 128 if j < 4 else 64
            blk = jnp.concatenate(parts, axis=0).T
            wotp_ref[j * 64:j * 64 + n // 2, :] = _pk(blk[:n].astype(BF16))

    def bias_rows(off):
        r = jax.lax.broadcasted_iota(jnp.int32, (KP - D, TF), 0)
        b = b1_ref[pl.ds(off, TF)].astype(F32).reshape(1, TF)
        return jnp.where(r < 2, jnp.broadcast_to(b, (KP - D, TF)), 0.0).astype(BF16)

    def layernorm(b):
        x = xbuf[b].astype(F32)
        mu = jnp.sum(x, axis=0, keepdims=True) * (1.0 / D)
        xc = x - mu
        var = jnp.sum(xc * xc, axis=0, keepdims=True) * (1.0 / D)
        xn = xc * (jax.lax.rsqrt(var + EPS) * LOG2E)
        r = jax.lax.broadcasted_iota(jnp.int32, (KP - D, RB), 0)
        pad = jnp.where(r == 0, L2E_HI, jnp.where(r == 1, L2E_LO, 0.0))
        xn_ref[b] = _pk(jnp.concatenate([xn, pad], axis=0).T.astype(BF16))

    def dense1(b, w1c):
        return jnp.dot(_upk(xn_ref[b]), w1c, preferred_element_type=F32)

    def mish(h):
        e = jnp.exp2(jnp.minimum(h, 30.0))
        n = e * (e + 2.0)
        return ((h * n) * pl.reciprocal(n + 2.0, approx=True)).astype(BF16)

    def dense2(act, w2c):
        return jax.lax.dot_general(w2c, act, NT, preferred_element_type=F32)

    def attention(r0, blk):
        qs = jnp.concatenate([fz_ref[1]] * (RC // 8), axis=0)
        q = [q_ref[i, r0:r0 + RC, :] * qs for i in range(5)]
        logits = []
        for w in range(W):
            lo = HALO + r0 - DIL * w
            p = q[0] * kv_ref[0, lo:lo + RC, :]
            for i in range(1, 4):
                p = p + q[i] * kv_ref[i, lo:lo + RC, :]
            p = p + q[4] * kv_ref[8, lo:lo + RC, :]
            p = p + pltpu.roll(p, 64, 1)
            p = p + pltpu.roll(p, 32, 1)
            if r0 < DIL * w:
                pos = blk * RB + r0 + jax.lax.broadcasted_iota(jnp.int32, (RC, 128), 0)
                p = jnp.where(pos >= DIL * w, p, -1e9)
            logits.append(p)
        m = logits[0]
        for w in range(1, W):
            m = jnp.maximum(m, logits[w])
        e = [jnp.exp2(l - m) for l in logits]
        den = e[0]
        for w in range(1, W):
            den = den + e[w]
        inv = 1.0 / den
        done = None
        for i in range(5):
            plane = 4 + i if i < 4 else 8
            acc = None
            for w in range(W):
                lo = HALO + r0 - DIL * w
                t = e[w] * kv_ref[plane, lo:lo + RC, :]
                acc = t if acc is None else acc + t
            o = (acc * inv).astype(BF16)
            oa_ref[blk, r0:r0 + RC, i * 128:(i + 1) * 128] = o
            done = o if done is None else jnp.maximum(done, o)
        return done

    @pl.when(step == 0)
    def _first():
        xc = [x_copy(i) for i in range(NB)]
        u = [w1_first(i) for i in range(2)]
        v = [w2_first(i) for i in range(2)]
        wq_c = copy(wqkv_hbm, wq_raw, sems.at[SWQ])
        wo_c = copy(wo_hbm, wo_raw, sems.at[SWO])
        b1_c = copy(b1_hbm, b1_ref, sems.at[SB])
        for cp in (xc[0], xc[1], b1_c, u[0], u[1], v[0], v[1], xc[2], xc[3], xc[4], wq_c, xc[5], wo_c,
                   xc[6], xc[7]) + w_mid(0):
            cp.start()
        zs_ref[0] = 0
        fz_ref[1] = jnp.full((8, 128), (DH ** -0.5) / LOG2E, F32)
        kv_ref[:, RB:RB + HALO, :] = jnp.zeros((9, HALO, 128), F32)
        fz_ref[2] = jnp.ones((8, 128), F32)
        lo, hi = slice(0, TF // 2), slice(TF // 2, TF)

        def ffn1(b):
            return mish(dense1(b, w1f[...]))

        def ffn2(b, act):
            t = dense2(act, w2f[...])
            acc_ref[b] = t
            return t

        xc[0].wait()
        layernorm(0)
        for cp in (xc[1], b1_c, u[0]):
            cp.wait()
        layernorm(1)
        w1f[D:KP, :] = bias_rows(0)
        a0 = mish(dense1(0, w1f[:, lo]))
        h1 = dense1(1, w1f[:, lo])
        for cp in (u[1], v[0]):
            cp.wait()
        a1 = mish(h1)
        acc_ref[0] = dense2(a0, w2f[:, lo])
        a0 = mish(dense1(0, w1f[:, hi]))
        acc_ref[1] = dense2(a1, w2f[:, lo])
        h1 = dense1(1, w1f[:, hi])
        for cp in (v[1], xc[2], xc[3], xc[4]):
            cp.wait()
        a1 = mish(h1)
        for b in (2, 3, 4):
            layernorm(b)
        for c in range(NM):
            w1m[c, D:KP, :] = bias_rows(TF + c * TF)
        acc_ref[0] = acc_ref[0] + dense2(a0, w2f[:, hi])
        a2 = ffn1(2)
        acc_ref[1] = acc_ref[1] + dense2(a1, w2f[:, hi])
        a3 = ffn1(3)
        ffn2(2, a2)
        a4 = ffn1(4)
        ffn2(3, a3)
        for cp in (xc[5], wq_c, wo_c, xc[6], xc[7]):
            cp.wait()
        for b in (5, 6, 7):
            layernorm(b)
        t = ffn2(4, a4)
        release(t[96:104, 128:256])
        prep_wo()
        release(t[400:408, 128:256])
        prep_wqkv(2)
        a5 = ffn1(5)
        a6 = ffn1(6)
        t = ffn2(5, a5)
        release(t[96:104, 0:128])
        prep_wqkv(0)
        a7 = ffn1(7)
        t = ffn2(6, a6)
        release(t[96:104, 0:128])
        prep_wqkv(1)
        ffn2(7, a7)

    @pl.when(jnp.logical_and(step > 0, step <= NM))
    def _mid():
        c = step - 1
        for cp in w_mid(c):
            cp.wait()
        z = zs_ref[0]
        kv_ref[:, 0:HALO, :] = kv_ref[:, RB:RB + HALO, :]
        act = mish(dense1(0, w1m[c]))

        @pl.when(c < NM - 1)
        def _():
            for cp in w_mid(c + 1):
                cp.start()

        qkv = jax.lax.dot_general(_upk(wp_ref[...]), _upk(xn_ref[c]), NT, preferred_element_type=F32)
        for i in range(4):
            q_ref[i] = qkv[i * 128:(i + 1) * 128, :].T
            kv_ref[i, HALO:HALO + RB, :] = qkv[512 + i * 128:512 + (i + 1) * 128, :].T
            kv_ref[4 + i, HALO:HALO + RB, :] = qkv[1024 + i * 128:1024 + (i + 1) * 128, :].T
        q_ref[4] = jnp.concatenate([qkv[1536:1600, :], jnp.zeros((64, RB), F32)], axis=0).T
        kv_ref[8, HALO:HALO + RB, :] = qkv[1600:1728, :].T

        done = []

        def run_chunks(n):
            for _ in range(n):
                done.append(attention(len(done) * RC, c))

        run_chunks(RELEASE[0])
        for b in range(NB):
            if b + 1 < NB:
                nact = mish(dense1(b + 1, w1m[c]))
            else:
                d = done[0]
                for d2 in done[1:]:
                    d = jnp.maximum(d, d2)
                top = jnp.concatenate([jnp.where(z == 0, act[0:RC, 0:128], d), act[0:RC, 128:]], axis=1)
                act = jnp.concatenate([top, act[RC:]], axis=0)
            t = dense2(act, w2m[c])
            acc_ref[b] = acc_ref[b] + t
            for pt in range(4):
                g = 1 + 4 * b + pt
                if g < len(RELEASE) and RELEASE[g] > 0:
                    r, half = REL_ROWS[pt % 2], pt // 2
                    fz_ref[z] = t[r:r + 8, half * 128:half * 128 + 128]
                    run_chunks(RELEASE[g])
            act = nact

    @pl.when(step == NM + 1)
    def _last():
        def finish(b, cs):
            t = jax.lax.dot_general(_upk(wotp_ref[...]), oa_ref[b, cs, :], NT, preferred_element_type=F32)
            obuf[b, :, cs] = (xbuf[b, :, cs].astype(F32) + (acc_ref[b, :, cs] + t) * LN2).astype(BF16)

        for b in range(NB - 1):
            finish(b, slice(0, RB))
            o_copy(b).start()
        for i in range(2):
            finish(NB - 1, slice(i * 128, (i + 1) * 128))
            o_half(i).start()
        for b in range(NB - 1):
            o_copy(b).wait()
        for i in range(2):
            o_half(i).wait()


@jax.jit
def pallas_parallel_sum__sliding_local_dilated__dense_activation_mish__prompt_kernel(
    A_x: jax.Array,
    A_wqkv: jax.Array,
    A_wo: jax.Array,
    B_x: jax.Array,
    B_w1: jax.Array,
    B_b1: jax.Array,
    B_w2: jax.Array,
):
    del B_x
    hbm = pl.BlockSpec(memory_space=pl.ANY)
    out_t = pl.pallas_call(
        _kernel,
        grid=(NM + 2,),
        in_specs=[hbm] * 6,
        out_specs=hbm,
        out_shape=jax.ShapeDtypeStruct((D, S), BF16),
        scratch_shapes=[
            pltpu.VMEM((NB, D, RB), BF16),
            pltpu.VMEM((NB, RB // 2, KP), U32),
            pltpu.VMEM((KP, TF), BF16),
            pltpu.VMEM((NM, KP, TF), BF16),
            pltpu.VMEM((D, TF), BF16),
            pltpu.VMEM((NM, D, TF), BF16),
            pltpu.VMEM((D, 3 * D), BF16),
            pltpu.VMEM((D, D), BF16),
            pltpu.VMEM((F,), BF16),
            pltpu.VMEM((3 * D // 2, KP), U32),
            pltpu.VMEM((D // 2, KP), U32),
            pltpu.VMEM((3, NQ, 128), U32),
            pltpu.VMEM((5, D, 128), F32),
            pltpu.VMEM((NB, D, RB), F32),
            pltpu.VMEM((NB, D, RB), BF16),
            pltpu.VMEM((9, RB + HALO, 128), F32),
            pltpu.VMEM((5, RB, 128), F32),
            pltpu.VMEM((NB, RB, KP), BF16),
            pltpu.VMEM((3, 8, 128), F32),
            pltpu.SMEM((1,), jnp.int32),
            pltpu.SemaphoreType.DMA((NSEM,)),
        ],
        compiler_params=pltpu.CompilerParams(
            dimension_semantics=("arbitrary",), vmem_limit_bytes=100 * 1024 * 1024),
        name="fused",
    )(A_x.reshape(S, D).T, A_wqkv, A_wo, B_w1, B_b1, B_w2.T)
    return out_t.T.reshape(1, S, D)
```

```python
import jax
import jax.numpy as jnp
import jax.experimental.pallas as pl
import jax.experimental.pallas.tpu as pltpu

S, D, F = 2048, 576, 4608
H, DH, W, DIL = 32, 18, 8, 2
KP = 640
NQ = 14 * 128
HALO = 16
RB = 256
NB = S // RB
TF = 512
NM = F // TF - 1
RC = 16
EPS = 1e-5
LOG2E = 1.4426950408889634
LN2 = 0.6931471805599453
L2E_HI = 1.4453125
L2E_LO = -0.00262451171875
NT = (((1,), (1,)), ((), ()))
F32, BF16, U32 = jnp.float32, jnp.bfloat16, jnp.uint32

RELEASE = [1, 1, 1, 1, 1, 0, 1, 1, 1] + [0, 1, 1, 0] * 4
REL_ROWS = (96, 400)

SX = 0
SW1 = SX + NB
SW2 = SW1 + NM + 2
SWQ = SW2 + NM + 2
SWO, SB, SO = SWQ + 1, SWQ + 2, SWQ + 3
TAIL = [(0, 256), (256, 192), (448, 128)]
NSEM = SO + NB + len(TAIL)


def _pk(v):
    return pltpu.bitcast(v, U32)


def _upk(v):
    return pltpu.bitcast(v, BF16)


def _kernel(xt_hbm, wqkv_hbm, wo_hbm, w1_hbm, b1_hbm, w2t_hbm, out_hbm,
            xbuf, xn_ref, w1f, w1m, w2f, w2m, wq_raw, wo_raw, b1_ref, wp_ref, wotp_ref,
            t_ref, wo32_ref, acc_ref, obuf, kv_ref, q_ref, oa_ref, fz_ref, zs_ref, sems):
    step = pl.program_id(0)
    copy = pltpu.make_async_copy

    def x_copy(i):
        return copy(xt_hbm.at[:, pl.ds(i * RB, RB)], xbuf.at[i], sems.at[SX + i])

    def o_copy(i):
        return copy(obuf.at[i], out_hbm.at[:, pl.ds(i * RB, RB)], sems.at[SO + i])

    def w1_first(i):
        cs = pl.ds(i * (TF // 2), TF // 2)
        return copy(w1_hbm.at[:, cs], w1f.at[pl.ds(0, D), cs], sems.at[SW1 + NM + i])

    def w2_first(i):
        cs = pl.ds(i * (TF // 2), TF // 2)
        return copy(w2t_hbm.at[:, cs], w2f.at[:, cs], sems.at[SW2 + NM + i])

    def w_mid(c):
        off = TF + c * TF
        if not isinstance(c, int):
            off = pl.multiple_of(off, 128)
        return (copy(w1_hbm.at[:, pl.ds(off, TF)], w1m.at[c, pl.ds(0, D), :], sems.at[SW1 + c]),
                copy(w2t_hbm.at[:, pl.ds(off, TF)], w2m.at[c], sems.at[SW2 + c]))

    def release(v):
        fz_ref[zs_ref[0]] = v

    def prep_wqkv(j):
        one = fz_ref[2, 0:1, 0:1]
        if j < 2:
            lo = wq_raw[j * 256:j * 256 + 128, :].astype(F32) * one
            hi = wq_raw[j * 256 + 128:j * 256 + 256, :].astype(F32)
            wq = _pk(pltpu.pack_elementwise([lo, hi], packed_dtype=BF16))
        else:
            hi = wq_raw[512:D, :].astype(F32) * one
            wq = jnp.concatenate([_pk(hi), jnp.zeros((64, 3 * D), U32)], axis=0)
        wq = jnp.concatenate([wq, jnp.zeros((128, NQ - 3 * D), U32)], axis=1)
        t_ref[j] = wq.T
        rows = lambda x, d: t_ref[j, pl.ds(x * D + d, H, stride=DH), :]
        parts = [rows(x, d) for x in range(3) for d in range(16)]
        parts += [rows(x, d) for x in range(3) for d in (16, 17)]
        u = jnp.concatenate(parts, axis=0)
        if j < 2:
            tiles = [(2 * j, pltpu.bitcast(u << 16, F32)),
                     (2 * j + 1, pltpu.bitcast(u & jnp.uint32(0xFFFF0000), F32))]
        else:
            tiles = [(4, pltpu.bitcast(u, F32))]
        for kt, v in tiles:
            wp_ref[:, kt * 128:(kt + 1) * 128] = _pk(v.astype(BF16))

    def prep_wo():
        wo = wo_raw[...].astype(F32)
        wo = jnp.concatenate([wo, jnp.zeros((D, KP - D), F32)], axis=1)
        for j in range(5):
            wo32_ref[j] = wo[:, j * 128:(j + 1) * 128]
        for j in range(5):
            rows = lambda d: wo32_ref[j, pl.ds(d, H, stride=DH), :]
            parts = [rows(d) for d in range(16)] + [jnp.zeros((64, 128), F32), rows(16), rows(17)]
            n = 128 if j < 4 else 64
            blk = jnp.concatenate(parts, axis=0).T
            wotp_ref[j * 64:j * 64 + n // 2, :] = _pk(blk[:n].astype(BF16))

    def bias_rows(off):
        r = jax.lax.broadcasted_iota(jnp.int32, (KP - D, TF), 0)
        b = b1_ref[pl.ds(off, TF)].astype(F32).reshape(1, TF)
        return jnp.where(r < 2, jnp.broadcast_to(b, (KP - D, TF)), 0.0).astype(BF16)

    def layernorm(b):
        x = xbuf[b].astype(F32)
        mu = jnp.sum(x, axis=0, keepdims=True) * (1.0 / D)
        xc = x - mu
        var = jnp.sum(xc * xc, axis=0, keepdims=True) * (1.0 / D)
        xn = xc * (jax.lax.rsqrt(var + EPS) * LOG2E)
        r = jax.lax.broadcasted_iota(jnp.int32, (KP - D, RB), 0)
        pad = jnp.where(r == 0, L2E_HI, jnp.where(r == 1, L2E_LO, 0.0))
        xn_ref[b] = _pk(jnp.concatenate([xn, pad], axis=0).T.astype(BF16))

    def dense1(b, w1c):
        return jnp.dot(_upk(xn_ref[b]), w1c, preferred_element_type=F32)

    def mish(h):
        e = jnp.exp2(jnp.minimum(h, 30.0))
        n = e * (e + 2.0)
        return ((h * n) * pl.reciprocal(n + 2.0, approx=True)).astype(BF16)

    def dense2(act, w2c):
        return jax.lax.dot_general(w2c, act, NT, preferred_element_type=F32)

    def attention(r0, blk):
        qs = jnp.concatenate([fz_ref[1]] * (RC // 8), axis=0)
        q = [q_ref[i, r0:r0 + RC, :] * qs for i in range(5)]
        logits = []
        for w in range(W):
            lo = HALO + r0 - DIL * w
            p = q[0] * kv_ref[0, lo:lo + RC, :]
            for i in range(1, 4):
                p = p + q[i] * kv_ref[i, lo:lo + RC, :]
            p = p + q[4] * kv_ref[8, lo:lo + RC, :]
            p = p + pltpu.roll(p, 64, 1)
            p = p + pltpu.roll(p, 32, 1)
            if r0 < DIL * w:
                pos = blk * RB + r0 + jax.lax.broadcasted_iota(jnp.int32, (RC, 128), 0)
                p = jnp.where(pos >= DIL * w, p, -1e9)
            logits.append(p)
        m = logits[0]
        for w in range(1, W):
            m = jnp.maximum(m, logits[w])
        e = [jnp.exp2(l - m) for l in logits]
        den = e[0]
        for w in range(1, W):
            den = den + e[w]
        inv = 1.0 / den
        done = None
        for i in range(5):
            plane = 4 + i if i < 4 else 8
            acc = None
            for w in range(W):
                lo = HALO + r0 - DIL * w
                t = e[w] * kv_ref[plane, lo:lo + RC, :]
                acc = t if acc is None else acc + t
            o = (acc * inv).astype(BF16)
            oa_ref[blk, r0:r0 + RC, i * 128:(i + 1) * 128] = o
            done = o if done is None else jnp.maximum(done, o)
        return done

    @pl.when(step == 0)
    def _first():
        xc = [x_copy(i) for i in range(NB)]
        u = [w1_first(i) for i in range(2)]
        v = [w2_first(i) for i in range(2)]
        wq_c = copy(wqkv_hbm, wq_raw, sems.at[SWQ])
        wo_c = copy(wo_hbm, wo_raw, sems.at[SWO])
        b1_c = copy(b1_hbm, b1_ref, sems.at[SB])
        for cp in (xc[0], xc[1], b1_c, u[0], u[1], v[0], v[1], xc[2], xc[3], xc[4], wq_c, xc[5], wo_c,
                   xc[6], xc[7]) + w_mid(0):
            cp.start()
        zs_ref[0] = 0
        fz_ref[1] = jnp.full((8, 128), (DH ** -0.5) / LOG2E, F32)
        kv_ref[:, RB:RB + HALO, :] = jnp.zeros((9, HALO, 128), F32)
        fz_ref[2] = jnp.ones((8, 128), F32)
        lo, hi = slice(0, TF // 2), slice(TF // 2, TF)

        def ffn1(b):
            return mish(dense1(b, w1f[...]))

        def ffn2(b, act):
            t = dense2(act, w2f[...])
            acc_ref[b] = t
            return t

        xc[0].wait()
        layernorm(0)
        for cp in (xc[1], b1_c, u[0]):
            cp.wait()
        layernorm(1)
        w1f[D:KP, :] = bias_rows(0)
        a0 = mish(dense1(0, w1f[:, lo]))
        h1 = dense1(1, w1f[:, lo])
        for cp in (u[1], v[0]):
            cp.wait()
        a1 = mish(h1)
        acc_ref[0] = dense2(a0, w2f[:, lo])
        a0 = mish(dense1(0, w1f[:, hi]))
        acc_ref[1] = dense2(a1, w2f[:, lo])
        h1 = dense1(1, w1f[:, hi])
        for cp in (v[1], xc[2], xc[3], xc[4]):
            cp.wait()
        a1 = mish(h1)
        for b in (2, 3, 4):
            layernorm(b)
        for c in range(NM):
            w1m[c, D:KP, :] = bias_rows(TF + c * TF)
        acc_ref[0] = acc_ref[0] + dense2(a0, w2f[:, hi])
        a2 = ffn1(2)
        acc_ref[1] = acc_ref[1] + dense2(a1, w2f[:, hi])
        a3 = ffn1(3)
        ffn2(2, a2)
        a4 = ffn1(4)
        ffn2(3, a3)
        for cp in (xc[5], wq_c, wo_c, xc[6], xc[7]):
            cp.wait()
        for b in (5, 6, 7):
            layernorm(b)
        prep_wo()
        ffn2(4, a4)
        a5 = ffn1(5)
        a6 = ffn1(6)
        t = ffn2(5, a5)
        release(t[96:104, 0:128])
        prep_wqkv(0)
        release(t[96:104, 128:256])
        prep_wqkv(2)
        a7 = ffn1(7)
        t = ffn2(6, a6)
        release(t[96:104, 0:128])
        prep_wqkv(1)
        ffn2(7, a7)

    @pl.when(jnp.logical_and(step > 0, step <= NM))
    def _mid():
        c = step - 1
        for cp in w_mid(c):
            cp.wait()
        z = zs_ref[0]
        kv_ref[:, 0:HALO, :] = kv_ref[:, RB:RB + HALO, :]
        act = mish(dense1(0, w1m[c]))

        @pl.when(c < NM - 1)
        def _():
            for cp in w_mid(c + 1):
                cp.start()

        qkv = jax.lax.dot_general(_upk(wp_ref[...]), _upk(xn_ref[c]), NT, preferred_element_type=F32)
        for i in range(4):
            q_ref[i] = qkv[i * 128:(i + 1) * 128, :].T
            kv_ref[i, HALO:HALO + RB, :] = qkv[512 + i * 128:512 + (i + 1) * 128, :].T
            kv_ref[4 + i, HALO:HALO + RB, :] = qkv[1024 + i * 128:1024 + (i + 1) * 128, :].T
        q_ref[4] = jnp.concatenate([qkv[1536:1600, :], jnp.zeros((64, RB), F32)], axis=0).T
        kv_ref[8, HALO:HALO + RB, :] = qkv[1600:1728, :].T

        done = []

        def run_chunks(n):
            for _ in range(n):
                done.append(attention(len(done) * RC, c))

        run_chunks(RELEASE[0])
        for b in range(NB):
            if b + 1 < NB:
                nact = mish(dense1(b + 1, w1m[c]))
            else:
                d = done[0]
                for d2 in done[1:]:
                    d = jnp.maximum(d, d2)
                top = jnp.concatenate([jnp.where(z == 0, act[0:RC, 0:128], d), act[0:RC, 128:]], axis=1)
                act = jnp.concatenate([top, act[RC:]], axis=0)
            t = dense2(act, w2m[c])
            acc_ref[b] = acc_ref[b] + t
            for pt in range(4):
                g = 1 + 4 * b + pt
                if g < len(RELEASE) and RELEASE[g] > 0:
                    r, half = REL_ROWS[pt % 2], pt // 2
                    fz_ref[z] = t[r:r + 8, half * 128:half * 128 + 128]
                    run_chunks(RELEASE[g])
            act = nact

    @pl.when(step == NM + 1)
    def _last():
        def project(b, cs):
            return jax.lax.dot_general(_upk(wotp_ref[...]), oa_ref[b, cs, :], NT, preferred_element_type=F32)

        def finish(b, rs, cs, t):
            obuf[b, rs, cs] = (xbuf[b, rs, cs].astype(F32) + (acc_ref[b, rs, cs] + t) * LN2).astype(BF16)

        def piece(k, r0, nr, c0, nc):
            return copy(obuf.at[NB - 1, pl.ds(r0, nr), pl.ds(c0, nc)],
                        out_hbm.at[pl.ds(r0, nr), pl.ds((NB - 1) * RB + c0, nc)], sems.at[SO + NB - 1 + k])

        full = slice(0, D)
        for b in range(NB - 1):
            finish(b, full, slice(0, RB), project(b, slice(0, RB)))
            o_copy(b).start()
        finish(NB - 1, full, slice(0, 128), project(NB - 1, slice(0, 128)))
        piece(0, 0, D, 0, 128).start()
        t = project(NB - 1, slice(128, RB))
        for k, (r0, nr) in enumerate(TAIL):
            finish(NB - 1, slice(r0, r0 + nr), slice(128, RB), t[r0:r0 + nr])
            piece(1 + k, r0, nr, 128, 128).start()
        for b in range(NB - 1):
            o_copy(b).wait()
        piece(0, 0, D, 0, 128).wait()
        for k, (r0, nr) in enumerate(TAIL):
            piece(1 + k, r0, nr, 128, 128).wait()


@jax.jit
def pallas_parallel_sum__sliding_local_dilated__dense_activation_mish__prompt_kernel(
    A_x: jax.Array,
    A_wqkv: jax.Array,
    A_wo: jax.Array,
    B_x: jax.Array,
    B_w1: jax.Array,
    B_b1: jax.Array,
    B_w2: jax.Array,
):
    del B_x
    hbm = pl.BlockSpec(memory_space=pl.ANY)
    out_t = pl.pallas_call(
        _kernel,
        grid=(NM + 2,),
        in_specs=[hbm] * 6,
        out_specs=hbm,
        out_shape=jax.ShapeDtypeStruct((D, S), BF16),
        scratch_shapes=[
            pltpu.VMEM((NB, D, RB), BF16),
            pltpu.VMEM((NB, RB // 2, KP), U32),
            pltpu.VMEM((KP, TF), BF16),
            pltpu.VMEM((NM, KP, TF), BF16),
            pltpu.VMEM((D, TF), BF16),
            pltpu.VMEM((NM, D, TF), BF16),
            pltpu.VMEM((D, 3 * D), BF16),
            pltpu.VMEM((D, D), BF16),
            pltpu.VMEM((F,), BF16),
            pltpu.VMEM((3 * D // 2, KP), U32),
            pltpu.VMEM((D // 2, KP), U32),
            pltpu.VMEM((3, NQ, 128), U32),
            pltpu.VMEM((5, D, 128), F32),
            pltpu.VMEM((NB, D, RB), F32),
            pltpu.VMEM((NB, D, RB), BF16),
            pltpu.VMEM((9, RB + HALO, 128), F32),
            pltpu.VMEM((5, RB, 128), F32),
            pltpu.VMEM((NB, RB, KP), BF16),
            pltpu.VMEM((3, 8, 128), F32),
            pltpu.SMEM((1,), jnp.int32),
            pltpu.SemaphoreType.DMA((NSEM,)),
        ],
        compiler_params=pltpu.CompilerParams(
            dimension_semantics=("arbitrary",), vmem_limit_bytes=100 * 1024 * 1024),
        name="fused",
    )(A_x.reshape(S, D).T, A_wqkv, A_wo, B_w1, B_b1, B_w2.T)
    return out_t.T.reshape(1, S, D)
```

```python
import jax
import jax.numpy as jnp
import jax.experimental.pallas as pl
import jax.experimental.pallas.tpu as pltpu

S, D, F = 2048, 576, 4608
H, DH, W, DIL = 32, 18, 8, 2
KP = 640
NQ = 14 * 128
HALO = 16
RB = 256
NB = S // RB
TF = 512
NM = F // TF - 1
RC = 16
EPS = 1e-5
LOG2E = 1.4426950408889634
LN2 = 0.6931471805599453
L2E_HI = 1.4453125
L2E_LO = -0.00262451171875
NT = (((1,), (1,)), ((), ()))
F32, BF16, U32 = jnp.float32, jnp.bfloat16, jnp.uint32

RELEASE = [1, 1, 1, 1, 1, 0, 1, 1, 1] + [0, 1, 1, 0] * 4
REL_ROWS = (96, 400)

TAIL = [(0, 256), (256, 192), (448, 128)]

X_SEM = (0, 1, 3, 3, 3, 1, 1, 1)
W1_SEM, W2_SEM = (1, 2), (2, 3)
B1_SEM, WQ_SEM, WO_SEM, MID_SEM, OUT_SEM = 1, 1, 1, 0, 0
NSEM = 4


def _pk(v):
    return pltpu.bitcast(v, U32)


def _upk(v):
    return pltpu.bitcast(v, BF16)


def _kernel(xt_hbm, wqkv_hbm, wo_hbm, w1_hbm, b1_hbm, w2t_hbm, out_hbm,
            xbuf, xn_ref, w1f, w1m, w2f, w2m, wq_raw, wo_raw, b1_ref, wp_ref, wotp_ref,
            t_ref, wo32_ref, acc_ref, obuf, kv_ref, q_ref, oa_ref, fz_ref, zs_ref, sems):
    step = pl.program_id(0)
    copy = pltpu.make_async_copy

    def x_copy(i):
        return copy(xt_hbm.at[:, pl.ds(i * RB, RB)], xbuf.at[i], sems.at[X_SEM[i]])

    def o_copy(i):
        return copy(obuf.at[i], out_hbm.at[:, pl.ds(i * RB, RB)], sems.at[OUT_SEM])

    def w1_first(i):
        cs = pl.ds(i * (TF // 2), TF // 2)
        return copy(w1_hbm.at[:, cs], w1f.at[pl.ds(0, D), cs], sems.at[W1_SEM[i]])

    def w2_first(i):
        cs = pl.ds(i * (TF // 2), TF // 2)
        return copy(w2t_hbm.at[:, cs], w2f.at[:, cs], sems.at[W2_SEM[i]])

    def w_mid(c):
        off = TF + c * TF
        if not isinstance(c, int):
            off = pl.multiple_of(off, 128)
        return (copy(w1_hbm.at[:, pl.ds(off, TF)], w1m.at[c, pl.ds(0, D), :], sems.at[MID_SEM]),
                copy(w2t_hbm.at[:, pl.ds(off, TF)], w2m.at[c], sems.at[MID_SEM]))

    def release(v):
        fz_ref[zs_ref[0]] = v

    def prep_wqkv(j):
        one = fz_ref[2, 0:1, 0:1]
        if j < 2:
            lo = wq_raw[j * 256:j * 256 + 128, :].astype(F32) * one
            hi = wq_raw[j * 256 + 128:j * 256 + 256, :].astype(F32)
            wq = (_pk(lo) >> 16) | _pk(hi)
        else:
            hi = wq_raw[512:D, :].astype(F32) * one
            wq = jnp.concatenate([_pk(hi), jnp.zeros((64, 3 * D), U32)], axis=0)
        wq = jnp.concatenate([wq, jnp.zeros((128, NQ - 3 * D), U32)], axis=1)
        t_ref[j] = wq.T
        rows = lambda x, d: t_ref[j, pl.ds(x * D + d, H, stride=DH), :]
        parts = [rows(x, d) for x in range(3) for d in range(16)]
        parts += [rows(x, d) for x in range(3) for d in (16, 17)]
        u = jnp.concatenate(parts, axis=0)
        if j < 2:
            tiles = [(2 * j, pltpu.bitcast(u << 16, F32)),
                     (2 * j + 1, pltpu.bitcast(u & jnp.uint32(0xFFFF0000), F32))]
        else:
            tiles = [(4, pltpu.bitcast(u, F32))]
        for kt, v in tiles:
            wp_ref[:, kt * 128:(kt + 1) * 128] = _pk(v.astype(BF16))

    def prep_wo():
        wo = wo_raw[...].astype(F32)
        wo = jnp.concatenate([wo, jnp.zeros((D, KP - D), F32)], axis=1)
        for j in range(5):
            wo32_ref[j] = wo[:, j * 128:(j + 1) * 128]
        for j in range(5):
            rows = lambda d: wo32_ref[j, pl.ds(d, H, stride=DH), :]
            parts = [rows(d) for d in range(16)] + [jnp.zeros((64, 128), F32), rows(16), rows(17)]
            n = 128 if j < 4 else 64
            blk = jnp.concatenate(parts, axis=0).T
            wotp_ref[j * 64:j * 64 + n // 2, :] = _pk(blk[:n].astype(BF16))

    def bias_rows(off):
        r = jax.lax.broadcasted_iota(jnp.int32, (KP - D, TF), 0)
        b = b1_ref[pl.ds(off, TF)].astype(F32).reshape(1, TF)
        return jnp.where(r < 2, jnp.broadcast_to(b, (KP - D, TF)), 0.0).astype(BF16)

    def layernorm(b):
        x = xbuf[b].astype(F32)
        mu = jnp.sum(x, axis=0, keepdims=True) * (1.0 / D)
        xc = x - mu
        var = jnp.sum(xc * xc, axis=0, keepdims=True) * (1.0 / D)
        xn = xc * (jax.lax.rsqrt(var + EPS) * LOG2E)
        r = jax.lax.broadcasted_iota(jnp.int32, (KP - D, RB), 0)
        pad = jnp.where(r == 0, L2E_HI, jnp.where(r == 1, L2E_LO, 0.0))
        xn_ref[b] = _pk(jnp.concatenate([xn, pad], axis=0).T.astype(BF16))

    def dense1(b, w1c):
        return jnp.dot(_upk(xn_ref[b]), w1c, preferred_element_type=F32)

    def mish(h):
        e = jnp.exp2(jnp.minimum(h, 30.0))
        n = e * (e + 2.0)
        return ((h * n) * pl.reciprocal(n + 2.0, approx=True)).astype(BF16)

    def dense2(act, w2c):
        return jax.lax.dot_general(w2c, act, NT, preferred_element_type=F32)

    def attention(r0, blk):
        qs = jnp.concatenate([fz_ref[1]] * (RC // 8), axis=0)
        q = [q_ref[i, r0:r0 + RC, :] * qs for i in range(5)]
        logits = []
        for w in range(W):
            lo = HALO + r0 - DIL * w
            p = q[0] * kv_ref[0, lo:lo + RC, :]
            for i in range(1, 4):
                p = p + q[i] * kv_ref[i, lo:lo + RC, :]
            p = p + q[4] * kv_ref[8, lo:lo + RC, :]
            p = p + pltpu.roll(p, 64, 1)
            p = p + pltpu.roll(p, 32, 1)
            if r0 < DIL * w:
                pos = blk * RB + r0 + jax.lax.broadcasted_iota(jnp.int32, (RC, 128), 0)
                p = jnp.where(pos >= DIL * w, p, -1e9)
            logits.append(p)
        m = logits[0]
        for w in range(1, W):
            m = jnp.maximum(m, logits[w])
        e = [jnp.exp2(l - m) for l in logits]
        den = e[0]
        for w in range(1, W):
            den = den + e[w]
        inv = 1.0 / den
        done = None
        for i in range(5):
            plane = 4 + i if i < 4 else 8
            acc = None
            for w in range(W):
                lo = HALO + r0 - DIL * w
                t = e[w] * kv_ref[plane, lo:lo + RC, :]
                acc = t if acc is None else acc + t
            o = (acc * inv).astype(BF16)
            oa_ref[blk, r0:r0 + RC, i * 128:(i + 1) * 128] = o
            done = o if done is None else jnp.maximum(done, o)
        return done

    @pl.when(step == 0)
    def _first():
        xc = [x_copy(i) for i in range(NB)]
        u = [w1_first(i) for i in range(2)]
        v = [w2_first(i) for i in range(2)]
        wq_c = copy(wqkv_hbm, wq_raw, sems.at[WQ_SEM])
        wo_c = copy(wo_hbm, wo_raw, sems.at[WO_SEM])
        b1_c = copy(b1_hbm, b1_ref, sems.at[B1_SEM])
        for cp in (xc[0], xc[1], b1_c, u[0], u[1], v[0], v[1], xc[2], xc[3], xc[4]):
            cp.start()
        zs_ref[0] = 0
        fz_ref[1] = jnp.full((8, 128), (DH ** -0.5) / LOG2E, F32)
        kv_ref[:, RB:RB + HALO, :] = jnp.zeros((9, HALO, 128), F32)
        fz_ref[2] = jnp.ones((8, 128), F32)
        lo, hi = slice(0, TF // 2), slice(TF // 2, TF)

        def ffn1(b):
            return mish(dense1(b, w1f[...]))

        def ffn2(b, act):
            t = dense2(act, w2f[...])
            acc_ref[b] = t
            return t

        xc[0].wait()
        layernorm(0)
        for cp in (xc[1], b1_c, u[0]):
            cp.wait()
        for cp in (wq_c, xc[5], wo_c, xc[6], xc[7]) + w_mid(0):
            cp.start()
        layernorm(1)
        w1f[D:KP, :] = bias_rows(0)
        a0 = mish(dense1(0, w1f[:, lo]))
        h1 = dense1(1, w1f[:, lo])
        for cp in (u[1], v[0]):
            cp.wait()
        a1 = mish(h1)
        acc_ref[0] = dense2(a0, w2f[:, lo])
        a0 = mish(dense1(0, w1f[:, hi]))
        acc_ref[1] = dense2(a1, w2f[:, lo])
        h1 = dense1(1, w1f[:, hi])
        for cp in (v[1], xc[2], xc[3], xc[4]):
            cp.wait()
        a1 = mish(h1)
        for b in (2, 3, 4):
            layernorm(b)
        for c in range(NM):
            w1m[c, D:KP, :] = bias_rows(TF + c * TF)
        acc_ref[0] = acc_ref[0] + dense2(a0, w2f[:, hi])
        a2 = ffn1(2)
        acc_ref[1] = acc_ref[1] + dense2(a1, w2f[:, hi])
        a3 = ffn1(3)
        ffn2(2, a2)
        a4 = ffn1(4)
        ffn2(3, a3)
        for cp in (xc[5], wq_c, wo_c, xc[6], xc[7]):
            cp.wait()
        for b in (5, 6, 7):
            layernorm(b)
        prep_wo()
        ffn2(4, a4)
        a5 = ffn1(5)
        a6 = ffn1(6)
        t = ffn2(5, a5)
        release(t[96:104, 0:128])
        prep_wqkv(0)
        release(t[96:104, 128:256])
        prep_wqkv(2)
        a7 = ffn1(7)
        t = ffn2(6, a6)
        release(t[96:104, 0:128])
        prep_wqkv(1)
        ffn2(7, a7)

    @pl.when(jnp.logical_and(step > 0, step <= NM))
    def _mid():
        c = step - 1
        for cp in w_mid(c):
            cp.wait()
        z = zs_ref[0]
        kv_ref[:, 0:HALO, :] = kv_ref[:, RB:RB + HALO, :]
        act = mish(dense1(0, w1m[c]))

        @pl.when(c < NM - 1)
        def _():
            for cp in w_mid(c + 1):
                cp.start()

        qkv = jax.lax.dot_general(_upk(wp_ref[...]), _upk(xn_ref[c]), NT, preferred_element_type=F32)
        for i in range(4):
            q_ref[i] = qkv[i * 128:(i + 1) * 128, :].T
            kv_ref[i, HALO:HALO + RB, :] = qkv[512 + i * 128:512 + (i + 1) * 128, :].T
            kv_ref[4 + i, HALO:HALO + RB, :] = qkv[1024 + i * 128:1024 + (i + 1) * 128, :].T
        q_ref[4] = jnp.concatenate([qkv[1536:1600, :], jnp.zeros((64, RB), F32)], axis=0).T
        kv_ref[8, HALO:HALO + RB, :] = qkv[1600:1728, :].T

        done = []

        def run_chunks(n):
            for _ in range(n):
                done.append(attention(len(done) * RC, c))

        run_chunks(RELEASE[0])
        for b in range(NB):
            if b + 1 < NB:
                nact = mish(dense1(b + 1, w1m[c]))
            else:
                d = done[0]
                for d2 in done[1:]:
                    d = jnp.maximum(d, d2)
                top = jnp.concatenate([jnp.where(z == 0, act[0:RC, 0:128], d), act[0:RC, 128:]], axis=1)
                act = jnp.concatenate([top, act[RC:]], axis=0)
            t = dense2(act, w2m[c])
            acc_ref[b] = acc_ref[b] + t
            for pt in range(4):
                g = 1 + 4 * b + pt
                if g < len(RELEASE) and RELEASE[g] > 0:
                    r, half = REL_ROWS[pt % 2], pt // 2
                    fz_ref[z] = t[r:r + 8, half * 128:half * 128 + 128]
                    run_chunks(RELEASE[g])
            act = nact

    @pl.when(step == NM + 1)
    def _last():
        def project(b, cs):
            return jax.lax.dot_general(_upk(wotp_ref[...]), oa_ref[b, cs, :], NT, preferred_element_type=F32)

        def finish(b, rs, cs, t):
            obuf[b, rs, cs] = (xbuf[b, rs, cs].astype(F32) + (acc_ref[b, rs, cs] + t) * LN2).astype(BF16)

        def piece(k, r0, nr, c0, nc):
            return copy(obuf.at[NB - 1, pl.ds(r0, nr), pl.ds(c0, nc)],
                        out_hbm.at[pl.ds(r0, nr), pl.ds((NB - 1) * RB + c0, nc)], sems.at[OUT_SEM])

        full = slice(0, D)
        for b in range(NB - 1):
            finish(b, full, slice(0, RB), project(b, slice(0, RB)))
            o_copy(b).start()
        finish(NB - 1, full, slice(0, 128), project(NB - 1, slice(0, 128)))
        piece(0, 0, D, 0, 128).start()
        t = project(NB - 1, slice(128, RB))
        for k, (r0, nr) in enumerate(TAIL):
            finish(NB - 1, slice(r0, r0 + nr), slice(128, RB), t[r0:r0 + nr])
            piece(1 + k, r0, nr, 128, 128).start()
        for b in range(NB - 1):
            o_copy(b).wait()
        piece(0, 0, D, 0, 128).wait()
        for k, (r0, nr) in enumerate(TAIL):
            piece(1 + k, r0, nr, 128, 128).wait()


@jax.jit
def pallas_parallel_sum__sliding_local_dilated__dense_activation_mish__prompt_kernel(
    A_x: jax.Array,
    A_wqkv: jax.Array,
    A_wo: jax.Array,
    B_x: jax.Array,
    B_w1: jax.Array,
    B_b1: jax.Array,
    B_w2: jax.Array,
):
    del B_x
    hbm = pl.BlockSpec(memory_space=pl.ANY)
    out_t = pl.pallas_call(
        _kernel,
        grid=(NM + 2,),
        in_specs=[hbm] * 6,
        out_specs=hbm,
        out_shape=jax.ShapeDtypeStruct((D, S), BF16),
        scratch_shapes=[
            pltpu.VMEM((NB, D, RB), BF16),
            pltpu.VMEM((NB, RB // 2, KP), U32),
            pltpu.VMEM((KP, TF), BF16),
            pltpu.VMEM((NM, KP, TF), BF16),
            pltpu.VMEM((D, TF), BF16),
            pltpu.VMEM((NM, D, TF), BF16),
            pltpu.VMEM((D, 3 * D), BF16),
            pltpu.VMEM((D, D), BF16),
            pltpu.VMEM((F,), BF16),
            pltpu.VMEM((3 * D // 2, KP), U32),
            pltpu.VMEM((D // 2, KP), U32),
            pltpu.VMEM((3, NQ, 128), U32),
            pltpu.VMEM((5, D, 128), F32),
            pltpu.VMEM((NB, D, RB), F32),
            pltpu.VMEM((NB, D, RB), BF16),
            pltpu.VMEM((9, RB + HALO, 128), F32),
            pltpu.VMEM((5, RB, 128), F32),
            pltpu.VMEM((NB, RB, KP), BF16),
            pltpu.VMEM((3, 8, 128), F32),
            pltpu.SMEM((1,), jnp.int32),
            pltpu.SemaphoreType.DMA((NSEM,)),
        ],
        compiler_params=pltpu.CompilerParams(
            dimension_semantics=("arbitrary",), vmem_limit_bytes=100 * 1024 * 1024),
        name="fused",
    )(A_x.reshape(S, D).T, A_wqkv, A_wo, B_w1, B_b1, B_w2.T)
    return out_t.T.reshape(1, S, D)
```

```python
import jax
import jax.numpy as jnp
import jax.experimental.pallas as pl
import jax.experimental.pallas.tpu as pltpu

S, D, F = 2048, 576, 4608
H, DH, W, DIL = 32, 18, 8, 2
KP = 640
NQ = 14 * 128
HALO = 16
RB = 256
NB = S // RB
TF = 512
NM = F // TF - 1
RC = 16
EPS = 1e-5
LOG2E = 1.4426950408889634
LN2 = 0.6931471805599453
L2E_HI = 1.4453125
L2E_LO = -0.00262451171875
NT = (((1,), (1,)), ((), ()))
F32, BF16, U32 = jnp.float32, jnp.bfloat16, jnp.uint32

RELEASE = [1, 1, 1, 1, 1, 0, 1, 1, 1] + [0, 1, 1, 0] * 4
REL_ROWS = (96, 400)

TAIL = [(0, 256), (256, 192), (448, 128)]

X_SEM = (0, 1, 3, 3, 3, 3, 1, 1)
W1_SEM, W2_SEM = (1, 2), (2, 3)
B1_SEM, WQ_SEM, WO_SEM, MID_SEM, OUT_SEM = 1, 1, 1, 0, 0
NSEM = 4


def _pk(v):
    return pltpu.bitcast(v, U32)


def _upk(v):
    return pltpu.bitcast(v, BF16)


def _kernel(xt_hbm, wqkv_hbm, wo_hbm, w1_hbm, b1_hbm, w2t_hbm, out_hbm,
            xbuf, xn_ref, w1f, w1m, w2f, w2m, wq_raw, wo_raw, b1_ref, wp_ref, wotp_ref,
            t_ref, wo32_ref, acc_ref, obuf, kv_ref, q_ref, oa_ref, fz_ref, zs_ref, sems):
    step = pl.program_id(0)
    copy = pltpu.make_async_copy

    def x_copy(i):
        return copy(xt_hbm.at[:, pl.ds(i * RB, RB)], xbuf.at[i], sems.at[X_SEM[i]])

    def o_copy(i):
        return copy(obuf.at[i], out_hbm.at[:, pl.ds(i * RB, RB)], sems.at[OUT_SEM])

    def w1_first(i):
        cs = pl.ds(i * (TF // 2), TF // 2)
        return copy(w1_hbm.at[:, cs], w1f.at[pl.ds(0, D), cs], sems.at[W1_SEM[i]])

    def w2_first(i):
        cs = pl.ds(i * (TF // 2), TF // 2)
        return copy(w2t_hbm.at[:, cs], w2f.at[:, cs], sems.at[W2_SEM[i]])

    def w_mid(c):
        off = TF + c * TF
        if not isinstance(c, int):
            off = pl.multiple_of(off, 128)
        return (copy(w1_hbm.at[:, pl.ds(off, TF)], w1m.at[c, pl.ds(0, D), :], sems.at[MID_SEM]),
                copy(w2t_hbm.at[:, pl.ds(off, TF)], w2m.at[c], sems.at[MID_SEM]))

    def release(v):
        fz_ref[zs_ref[0]] = v

    def prep_wqkv(j):
        one = fz_ref[2, 0:1, 0:1]
        if j < 2:
            lo = wq_raw[j * 256:j * 256 + 128, :].astype(F32) * one
            hi = wq_raw[j * 256 + 128:j * 256 + 256, :].astype(F32)
            wq = (_pk(lo) >> 16) | _pk(hi)
        else:
            hi = wq_raw[512:D, :].astype(F32) * one
            wq = jnp.concatenate([_pk(hi), jnp.zeros((64, 3 * D), U32)], axis=0)
        wq = jnp.concatenate([wq, jnp.zeros((128, NQ - 3 * D), U32)], axis=1)
        t_ref[j] = wq.T
        rows = lambda x, d: t_ref[j, pl.ds(x * D + d, H, stride=DH), :]
        parts = [rows(x, d) for x in range(3) for d in range(16)]
        parts += [rows(x, d) for x in range(3) for d in (16, 17)]
        u = jnp.concatenate(parts, axis=0)
        if j < 2:
            tiles = [(2 * j, pltpu.bitcast(u << 16, F32)),
                     (2 * j + 1, pltpu.bitcast(u & jnp.uint32(0xFFFF0000), F32))]
        else:
            tiles = [(4, pltpu.bitcast(u, F32))]
        for kt, v in tiles:
            wp_ref[:, kt * 128:(kt + 1) * 128] = _pk(v.astype(BF16))

    def prep_wo():
        wo = wo_raw[...].astype(F32) * fz_ref[2, 0:1, 0:1]
        wo = jnp.concatenate([wo, jnp.zeros((D, KP - D), F32)], axis=1)
        for j in range(5):
            wo32_ref[j] = wo[:, j * 128:(j + 1) * 128]
        for j in range(5):
            rows = lambda d: wo32_ref[j, pl.ds(d, H, stride=DH), :]
            parts = [rows(d) for d in range(16)] + [jnp.zeros((64, 128), F32), rows(16), rows(17)]
            n = 128 if j < 4 else 64
            blk = jnp.concatenate(parts, axis=0).T
            wotp_ref[j * 64:j * 64 + n // 2, :] = _pk(blk[:n].astype(BF16))

    def bias_rows(off):
        r = jax.lax.broadcasted_iota(jnp.int32, (KP - D, TF), 0)
        b = b1_ref[pl.ds(off, TF)].astype(F32).reshape(1, TF)
        return jnp.where(r < 2, jnp.broadcast_to(b, (KP - D, TF)), 0.0).astype(BF16)

    def layernorm(b):
        x = xbuf[b].astype(F32)
        mu = jnp.sum(x, axis=0, keepdims=True) * (1.0 / D)
        xc = x - mu
        var = jnp.sum(xc * xc, axis=0, keepdims=True) * (1.0 / D)
        xn = xc * (jax.lax.rsqrt(var + EPS) * LOG2E)
        r = jax.lax.broadcasted_iota(jnp.int32, (KP - D, RB), 0)
        pad = jnp.where(r == 0, L2E_HI, jnp.where(r == 1, L2E_LO, 0.0))
        xn_ref[b] = _pk(jnp.concatenate([xn, pad], axis=0).T.astype(BF16))

    def dense1(b, w1c):
        return jnp.dot(_upk(xn_ref[b]), w1c, preferred_element_type=F32)

    def mish(h):
        e = jnp.exp2(jnp.minimum(h, 30.0))
        n = e * (e + 2.0)
        return ((h * n) * pl.reciprocal(n + 2.0, approx=True)).astype(BF16)

    def dense2(act, w2c):
        return jax.lax.dot_general(w2c, act, NT, preferred_element_type=F32)

    def attention(r0, blk):
        qs = jnp.concatenate([fz_ref[1]] * (RC // 8), axis=0)
        q = [q_ref[i, r0:r0 + RC, :] * qs for i in range(5)]
        logits = []
        for w in range(W):
            lo = HALO + r0 - DIL * w
            p = q[0] * kv_ref[0, lo:lo + RC, :]
            for i in range(1, 4):
                p = p + q[i] * kv_ref[i, lo:lo + RC, :]
            p = p + q[4] * kv_ref[8, lo:lo + RC, :]
            p = p + pltpu.roll(p, 64, 1)
            p = p + pltpu.roll(p, 32, 1)
            if r0 < DIL * w:
                pos = blk * RB + r0 + jax.lax.broadcasted_iota(jnp.int32, (RC, 128), 0)
                p = jnp.where(pos >= DIL * w, p, -1e9)
            logits.append(p)
        m = logits[0]
        for w in range(1, W):
            m = jnp.maximum(m, logits[w])
        e = [jnp.exp2(l - m) for l in logits]
        den = e[0]
        for w in range(1, W):
            den = den + e[w]
        inv = 1.0 / den
        done = None
        for i in range(5):
            plane = 4 + i if i < 4 else 8
            acc = None
            for w in range(W):
                lo = HALO + r0 - DIL * w
                t = e[w] * kv_ref[plane, lo:lo + RC, :]
                acc = t if acc is None else acc + t
            o = (acc * inv).astype(BF16)
            oa_ref[blk, r0:r0 + RC, i * 128:(i + 1) * 128] = o
            done = o if done is None else jnp.maximum(done, o)
        return done

    @pl.when(step == 0)
    def _first():
        xc = [x_copy(i) for i in range(NB)]
        u = [w1_first(i) for i in range(2)]
        v = [w2_first(i) for i in range(2)]
        wq_c = copy(wqkv_hbm, wq_raw, sems.at[WQ_SEM])
        wo_c = copy(wo_hbm, wo_raw, sems.at[WO_SEM])
        b1_c = copy(b1_hbm, b1_ref, sems.at[B1_SEM])
        for cp in (xc[0], xc[1], b1_c, u[0], u[1], v[0], v[1], xc[2], xc[3], xc[4], xc[5]):
            cp.start()
        zs_ref[0] = 0
        fz_ref[1] = jnp.full((8, 128), (DH ** -0.5) / LOG2E, F32)
        kv_ref[:, RB:RB + HALO, :] = jnp.zeros((9, HALO, 128), F32)
        fz_ref[2] = jnp.ones((8, 128), F32)
        lo, hi = slice(0, TF // 2), slice(TF // 2, TF)

        def ffn1(b):
            return mish(dense1(b, w1f[...]))

        def ffn2(b, act):
            t = dense2(act, w2f[...])
            acc_ref[b] = t
            return t

        xc[0].wait()
        layernorm(0)
        for cp in (xc[1], b1_c, u[0]):
            cp.wait()
        for cp in (wq_c, wo_c, xc[6], xc[7]) + w_mid(0):
            cp.start()
        layernorm(1)
        w1f[D:KP, :] = bias_rows(0)
        a0 = mish(dense1(0, w1f[:, lo]))
        h1 = dense1(1, w1f[:, lo])
        for cp in (u[1], v[0]):
            cp.wait()
        a1 = mish(h1)
        acc_ref[0] = dense2(a0, w2f[:, lo])
        a0 = mish(dense1(0, w1f[:, hi]))
        acc_ref[1] = dense2(a1, w2f[:, lo])
        h1 = dense1(1, w1f[:, hi])
        for cp in (v[1], xc[2], xc[3], xc[4], xc[5]):
            cp.wait()
        a1 = mish(h1)
        for b in (2, 3, 4, 5):
            layernorm(b)
        for c in range(NM):
            w1m[c, D:KP, :] = bias_rows(TF + c * TF)
        acc_ref[0] = acc_ref[0] + dense2(a0, w2f[:, hi])
        a2 = ffn1(2)
        acc_ref[1] = acc_ref[1] + dense2(a1, w2f[:, hi])
        a3 = ffn1(3)
        ffn2(2, a2)
        a4 = ffn1(4)
        ffn2(3, a3)
        h5 = dense1(5, w1f[...])
        for cp in (wq_c, wo_c, xc[6], xc[7]):
            cp.wait()
        a5 = mish(h5)
        for b in (6, 7):
            layernorm(b)
        t = ffn2(4, a4)
        release(t[240:248, 128:256])
        prep_wqkv(2)
        release(t[480:488, 128:256])
        prep_wo()
        a6 = ffn1(6)
        t = ffn2(5, a5)
        release(t[240:248, 0:128])
        prep_wqkv(0)
        a7 = ffn1(7)
        t = ffn2(6, a6)
        release(t[240:248, 0:128])
        prep_wqkv(1)
        ffn2(7, a7)

    @pl.when(jnp.logical_and(step > 0, step <= NM))
    def _mid():
        c = step - 1
        for cp in w_mid(c):
            cp.wait()
        z = zs_ref[0]
        kv_ref[:, 0:HALO, :] = kv_ref[:, RB:RB + HALO, :]
        act = mish(dense1(0, w1m[c]))

        @pl.when(c < NM - 1)
        def _():
            for cp in w_mid(c + 1):
                cp.start()

        qkv = jax.lax.dot_general(_upk(wp_ref[...]), _upk(xn_ref[c]), NT, preferred_element_type=F32)
        for i in range(4):
            q_ref[i] = qkv[i * 128:(i + 1) * 128, :].T
            kv_ref[i, HALO:HALO + RB, :] = qkv[512 + i * 128:512 + (i + 1) * 128, :].T
            kv_ref[4 + i, HALO:HALO + RB, :] = qkv[1024 + i * 128:1024 + (i + 1) * 128, :].T
        q_ref[4] = jnp.concatenate([qkv[1536:1600, :], jnp.zeros((64, RB), F32)], axis=0).T
        kv_ref[8, HALO:HALO + RB, :] = qkv[1600:1728, :].T

        done = []

        def run_chunks(n):
            for _ in range(n):
                done.append(attention(len(done) * RC, c))

        run_chunks(RELEASE[0])
        for b in range(NB):
            if b + 1 < NB:
                nact = mish(dense1(b + 1, w1m[c]))
            else:
                d = done[0]
                for d2 in done[1:]:
                    d = jnp.maximum(d, d2)
                top = jnp.concatenate([jnp.where(z == 0, act[0:RC, 0:128], d), act[0:RC, 128:]], axis=1)
                act = jnp.concatenate([top, act[RC:]], axis=0)
            t = dense2(act, w2m[c])
            acc_ref[b] = acc_ref[b] + t
            for pt in range(4):
                g = 1 + 4 * b + pt
                if g < len(RELEASE) and RELEASE[g] > 0:
                    r, half = REL_ROWS[pt % 2], pt // 2
                    fz_ref[z] = t[r:r + 8, half * 128:half * 128 + 128]
                    run_chunks(RELEASE[g])
            act = nact

    @pl.when(step == NM + 1)
    def _last():
        def project(b, cs):
            return jax.lax.dot_general(_upk(wotp_ref[...]), oa_ref[b, cs, :], NT, preferred_element_type=F32)

        def finish(b, rs, cs, t):
            obuf[b, rs, cs] = (xbuf[b, rs, cs].astype(F32) + (acc_ref[b, rs, cs] + t) * LN2).astype(BF16)

        def piece(r0, nr, c0, nc):
            return copy(obuf.at[NB - 1, pl.ds(r0, nr), pl.ds(c0, nc)],
                        out_hbm.at[pl.ds(r0, nr), pl.ds((NB - 1) * RB + c0, nc)], sems.at[OUT_SEM])

        full = slice(0, D)
        for b in range(NB - 1):
            finish(b, full, slice(0, RB), project(b, slice(0, RB)))
            o_copy(b).start()
        finish(NB - 1, full, slice(0, 128), project(NB - 1, slice(0, 128)))
        piece(0, D, 0, 128).start()
        t = project(NB - 1, slice(128, RB))
        for r0, nr in TAIL:
            finish(NB - 1, slice(r0, r0 + nr), slice(128, RB), t[r0:r0 + nr])
            piece(r0, nr, 128, 128).start()
        for b in range(NB - 1):
            o_copy(b).wait()
        piece(0, D, 0, 128).wait()
        for r0, nr in TAIL:
            piece(r0, nr, 128, 128).wait()


@jax.jit
def pallas_parallel_sum__sliding_local_dilated__dense_activation_mish__prompt_kernel(
    A_x: jax.Array,
    A_wqkv: jax.Array,
    A_wo: jax.Array,
    B_x: jax.Array,
    B_w1: jax.Array,
    B_b1: jax.Array,
    B_w2: jax.Array,
):
    del B_x
    hbm = pl.BlockSpec(memory_space=pl.ANY)
    out_t = pl.pallas_call(
        _kernel,
        grid=(NM + 2,),
        in_specs=[hbm] * 6,
        out_specs=hbm,
        out_shape=jax.ShapeDtypeStruct((D, S), BF16),
        scratch_shapes=[
            pltpu.VMEM((NB, D, RB), BF16),
            pltpu.VMEM((NB, RB // 2, KP), U32),
            pltpu.VMEM((KP, TF), BF16),
            pltpu.VMEM((NM, KP, TF), BF16),
            pltpu.VMEM((D, TF), BF16),
            pltpu.VMEM((NM, D, TF), BF16),
            pltpu.VMEM((D, 3 * D), BF16),
            pltpu.VMEM((D, D), BF16),
            pltpu.VMEM((F,), BF16),
            pltpu.VMEM((3 * D // 2, KP), U32),
            pltpu.VMEM((D // 2, KP), U32),
            pltpu.VMEM((3, NQ, 128), U32),
            pltpu.VMEM((5, D, 128), F32),
            pltpu.VMEM((NB, D, RB), F32),
            pltpu.VMEM((NB, D, RB), BF16),
            pltpu.VMEM((9, RB + HALO, 128), F32),
            pltpu.VMEM((5, RB, 128), F32),
            pltpu.VMEM((NB, RB, KP), BF16),
            pltpu.VMEM((3, 8, 128), F32),
            pltpu.SMEM((1,), jnp.int32),
            pltpu.SemaphoreType.DMA((NSEM,)),
        ],
        compiler_params=pltpu.CompilerParams(
            dimension_semantics=("arbitrary",), vmem_limit_bytes=100 * 1024 * 1024),
        name="fused",
    )(A_x.reshape(S, D).T, A_wqkv, A_wo, B_w1, B_b1, B_w2.T)
    return out_t.T.reshape(1, S, D)
```
